```python
import os as _os
_os.environ.setdefault("JAX_PLATFORMS", "cpu")
import jax
import jax.numpy as jnp

def _softmax(x, axis=-1):
    return jax.nn.softmax(x, axis=axis)
def _gelu(x):
    return jax.nn.gelu(x, approximate=True)
def _silu(x):
    return jax.nn.silu(x)
def _sigmoid(x):
    return jax.nn.sigmoid(x)
def _layernorm(x, axis=-1, eps=1e-5):
    m = jnp.mean(x, axis=axis, keepdims=True)
    v = jnp.var(x, axis=axis, keepdims=True)
    return (x - m) / jnp.sqrt(v + eps)
def _scatter_add(tgt, idx, src, axis=0):
    return tgt.at[idx].add(src)
def _segment_sum(src, seg, n):
    return jax.ops.segment_sum(src, seg, n)
class _Rng:
    def __init__(self, key):
        self._k = key
    def _next(self):
        self._k, sub = jax.random.split(self._k)
        return sub
    def normal(self, shape):
        return jax.random.normal(self._next(), shape, dtype=jnp.bfloat16)
    def randint(self, lo, hi, shape):
        return jax.random.randint(self._next(), shape, lo, hi, dtype=jnp.int32)
    def uniform(self, shape, lo=0.0, hi=1.0):
        return jax.random.uniform(self._next(), shape, jnp.bfloat16, lo, hi)
    def permutation(self, n):
        return jax.random.permutation(self._next(), n)


kernel_name = 'gated_mix__gqa_block_cached__dense_activation_squared_relu__decode'

def setup_inputs():
    _rng = _Rng(jax.random.key(int.from_bytes(__import__("os").urandom(4), "little")))
    _w = (lambda a: (lambda t: t.astype(jnp.bfloat16) if jnp.issubdtype(t.dtype, jnp.floating) else t)(jnp.asarray(a)))
    def _A_setup():
        B, Sq, D = 4, 1, 512
        Hq, Hkv, Sk, Dh = 32, 8, 4096, 128
        assert Hq % Hkv == 0, (Hq, Hkv)
        return {
            "x": _w((lambda *s: _rng.normal(s) * 0.05)(B, Sq, D)),
            "k_cache": _w((lambda *s: _rng.normal(s) * 3.2)(B, Hkv, Sk, Dh)),
            "v_cache": _w((lambda *s: _rng.normal(s) * 1.6)(B, Hkv, Sk, Dh)),
            "wq": _w((lambda *s: _rng.normal(s) * 3.2)(D, Hq * Dh) * (D ** -0.5)),
            "wo": _w((lambda *s: _rng.normal(s) * 1.6)(Hq * Dh, D) * ((Hq * Dh) ** -0.5)),
        }
    _A_in = _A_setup()

    def _B_setup():
        B, S, D, F = 4, 1, 512, 1792
        return {
            "x": _w((lambda *s: _rng.normal(s) * 0.05)(B, S, D)),
            "w1": _w((lambda *s: _rng.normal(s) * 0.1)(D, F)),
            "b1": _w((lambda *s: _rng.normal(s) * 0.05)(F)),
            "w2": _w((lambda *s: _rng.normal(s) * 0.05)(F, D)),
            "b2": _w((lambda *s: _rng.normal(s) * 0.05)(D)),
        }
    _B_in = _B_setup()

    return {
        "A_x": _A_in["x"],
        "A_k_cache": _A_in["k_cache"],
        "A_v_cache": _A_in["v_cache"],
        "A_wq": _A_in["wq"],
        "A_wo": _A_in["wo"],
        "B_x": _B_in["x"],
        "B_w1": _B_in["w1"],
        "B_b1": _B_in["b1"],
        "B_w2": _B_in["w2"],
        "B_b2": _B_in["b2"],
        "gate_w": _w((lambda *s: _rng.normal(s) * 0.05)(512) * 16.0),
    }

def reference(A_x, A_k_cache, A_v_cache, A_wq, A_wo, B_x, B_w1, B_b1, B_w2, B_b2, gate_w):
    def _A_ref(x, k_cache, v_cache, wq, wo):
        B, Sq, D = x.shape
        Hq, Dh = 32, 128
        Hkv = k_cache.shape[1]
        rep = Hq // Hkv
        q = (lambda x, *d: x.transpose(*d))((x @ wq).reshape(B, Sq, Hq, Dh), 0, 2, 1, 3)
        k = jnp.repeat(k_cache, rep, axis=1)
        v = jnp.repeat(v_cache, rep, axis=1)
        scores = jnp.einsum("bhqd,bhkd->bhqk", q, k) * (Dh ** -0.5)
        p = _softmax(scores, axis=-1)
        o = jnp.einsum("bhqk,bhkd->bhqd", p, v)
        return (lambda x, *d: x.transpose(*d))(o, 0, 2, 1, 3).reshape(B, Sq, Hq * Dh) @ wo

    def _B_ref(x, w1, b1, w2, b2):
        h = jnp.einsum("bsd,df->bsf", x, w1) + b1
        zero = jnp.zeros_like(h)
        r = jnp.where(h > zero, h, zero)
        h = r * r
        out = jnp.einsum("bsf,fd->bsd", h, w2) + b2
        return out

    x = A_x
    g = _sigmoid((x * gate_w).sum(-1, keepdims=True))
    a = _A_ref(x, A_k_cache, A_v_cache, A_wq, A_wo)
    b = _B_ref(x, B_w1, B_b1, B_w2, B_b2)
    return g * a + (1 - g) * b
```

```python
import jax
import jax.numpy as jnp
from jax import lax
import jax.experimental.pallas as pl
import jax.experimental.pallas.tpu as pltpu

B, D, HQ, HKV, SK, DH, F = 4, 512, 32, 8, 4096, 128, 1792
REP = HQ // HKV
M = REP * B
LOG2E = 1.4426950408889634
NS = 4
WOC = 4
NU = B * HKV
WO_ROWS = (HQ * DH) // WOC


def _kernel(x_h, k_h, v_h, wq_h, wo_h, w1_h, b1_h, w2_h, b2_h, gw_h, o_ref,
            xb, b1b, b2b, gwb, wqb, wob, w1b, w2b, kb, vb, q_s, o_s, ksem, vsem, wsem):
    def kv_copies(u, slot):
        h = u // B
        b = u % B
        return (pltpu.make_async_copy(k_h.at[b, h], kb.at[slot], ksem.at[slot]),
                pltpu.make_async_copy(v_h.at[b, h], vb.at[slot], vsem.at[slot]))

    c_x = pltpu.make_async_copy(x_h, xb, wsem.at[0])
    c_wq = pltpu.make_async_copy(wq_h, wqb, wsem.at[1])
    c_b1 = pltpu.make_async_copy(b1_h, b1b, wsem.at[2])
    c_b2 = pltpu.make_async_copy(b2_h, b2b, wsem.at[3])
    c_gw = pltpu.make_async_copy(gw_h, gwb, wsem.at[4])
    c_w1 = pltpu.make_async_copy(w1_h, w1b, wsem.at[5])
    c_w2 = pltpu.make_async_copy(w2_h, w2b, wsem.at[6])

    def c_wo(c):
        return pltpu.make_async_copy(wo_h.at[pl.ds(c * WO_ROWS, WO_ROWS)],
                                     wob.at[pl.ds(c * WO_ROWS, WO_ROWS)], wsem.at[7 + c])

    c_wq.start()
    c_x.start()
    for u in range(NS - 1):
        ck, cv = kv_copies(u, u)
        ck.start()
        cv.start()
    c_b1.start()
    c_b2.start()
    c_gw.start()
    c_w1.start()
    c_w2.start()

    c_x.wait()
    x4 = xb[...].astype(jnp.float32)
    x16 = jnp.concatenate([x4] * REP, axis=0)
    x16b = x16.astype(jnp.bfloat16)

    c_wq.wait()
    rowq = lax.broadcasted_iota(jnp.int32, (M, DH), 0)
    for h in range(HKV):
        qh = jnp.dot(x16b, wqb[:, h * REP * DH:(h + 1) * REP * DH],
                     preferred_element_type=jnp.float32)
        sel = qh[:, 0:DH]
        for r in range(1, REP):
            sel = jnp.where(rowq // B == r, qh[:, r * DH:(r + 1) * DH], sel)
        q_s[h] = sel.astype(jnp.bfloat16)

    cexp = (DH ** -0.5) * LOG2E

    def unit(u, carry):
        slot = u % NS
        nxt = u + NS - 1

        @pl.when(nxt < NU)
        def _():
            ck, cv = kv_copies(nxt, nxt % NS)
            ck.start()
            cv.start()

        @pl.when(nxt >= NU)
        def _():
            for c in range(WOC):
                @pl.when(nxt - NU == c)
                def _():
                    c_wo(c).start()

        h = u // B
        b = u % B
        ck, cv = kv_copies(u, slot)
        ck.wait()
        s = lax.dot_general(q_s[h], kb[slot], (((1,), (1,)), ((), ())),
                            preferred_element_type=jnp.float32)
        m = jnp.max(s, axis=1, keepdims=True)
        p = jnp.exp2((s - m) * cexp)
        l = jnp.sum(p, axis=1, keepdims=True)
        cv.wait()
        o = jnp.dot(p.astype(jnp.bfloat16), vb[slot],
                    preferred_element_type=jnp.float32) / l

        @pl.when(b == 0)
        def _():
            o_s[h] = o

        @pl.when(b > 0)
        def _():
            o_s[h] = jnp.where(rowq % B == b, o, o_s[h])

        return carry

    lax.fori_loop(0, NU, unit, 0)
    for c in range(NS - 1, WOC):
        c_wo(c).start()

    c_w1.wait()
    c_b1.wait()
    hh = jnp.dot(x16b, w1b[...], preferred_element_type=jnp.float32)
    hh = hh + b1b[...].astype(jnp.float32).reshape(1, F)
    hh = hh.astype(jnp.bfloat16).astype(jnp.float32)
    r_ = jnp.maximum(hh, 0.0)
    h2 = (r_ * r_).astype(jnp.bfloat16)
    c_w2.wait()
    c_b2.wait()
    ffn = jnp.dot(h2, w2b[...], preferred_element_type=jnp.float32)
    ffn = ffn + b2b[...].astype(jnp.float32).reshape(1, D)

    c_gw.wait()
    gl = jnp.sum(x16 * gwb[...].astype(jnp.float32).reshape(1, D), axis=1, keepdims=True)
    g = jax.nn.sigmoid(gl)

    acc = jnp.zeros((M, D), jnp.float32)
    heads_per_c = WO_ROWS // DH
    for c in range(WOC):
        c_wo(c).wait()
        for j in range(heads_per_c):
            hq = c * heads_per_c + j
            h, r = hq // REP, hq % REP
            lhs = jnp.where(rowq // B == r, o_s[h], 0.0).astype(jnp.bfloat16)
            acc = acc + jnp.dot(lhs, wob[hq * DH:(hq + 1) * DH, :],
                                preferred_element_type=jnp.float32)
    a = acc[0:4] + acc[4:8] + acc[8:12] + acc[12:16]
    res = g[0:4] * a + (1.0 - g[0:4]) * ffn[0:4]
    o_ref[...] = res.astype(jnp.bfloat16)


@jax.jit
def pallas_gated_mix__gqa_block_cached__dense_activation_squared_relu__decode_kernel(
    A_x: jax.Array,
    A_k_cache: jax.Array,
    A_v_cache: jax.Array,
    A_wq: jax.Array,
    A_wo: jax.Array,
    B_x: jax.Array,
    B_w1: jax.Array,
    B_b1: jax.Array,
    B_w2: jax.Array,
    B_b2: jax.Array,
    gate_w: jax.Array,
):
    del B_x
    bf = jnp.bfloat16
    out = pl.pallas_call(
        _kernel,
        out_shape=jax.ShapeDtypeStruct((B, D), bf),
        in_specs=[pl.BlockSpec(memory_space=pl.ANY)] * 10,
        out_specs=pl.BlockSpec(memory_space=pltpu.VMEM),
        scratch_shapes=[
            pltpu.VMEM((B, D), bf), pltpu.VMEM((F,), bf), pltpu.VMEM((D,), bf), pltpu.VMEM((D,), bf),
            pltpu.VMEM((D, HQ * DH), bf), pltpu.VMEM((HQ * DH, D), bf),
            pltpu.VMEM((D, F), bf), pltpu.VMEM((F, D), bf),
            pltpu.VMEM((NS, SK, DH), bf), pltpu.VMEM((NS, SK, DH), bf),
            pltpu.VMEM((HKV, M, DH), bf), pltpu.VMEM((HKV, M, DH), jnp.float32),
            pltpu.SemaphoreType.DMA((NS,)), pltpu.SemaphoreType.DMA((NS,)),
            pltpu.SemaphoreType.DMA((7 + WOC,)),
        ],
        compiler_params=pltpu.CompilerParams(vmem_limit_bytes=100 * 1024 * 1024),
    )(A_x.reshape(B, D), A_k_cache, A_v_cache, A_wq, A_wo, B_w1, B_b1, B_w2, B_b2, gate_w)
    return out.reshape(B, 1, D)
```

```python
import jax
import jax.numpy as jnp
from jax import lax
import jax.experimental.pallas as pl
import jax.experimental.pallas.tpu as pltpu

B, D, HQ, HKV, SK, DH, F = 4, 512, 32, 8, 4096, 128, 1792
REP = HQ // HKV
M = REP * B
LOG2E = 1.4426950408889634

NSEM = 3
NSLOT = NSEM + 1
NU = HKV * B
PRE = 2
WO_ROWS = (1664, 1024, 640, 384, 256, 128)
WOC = len(WO_ROWS)
WO_OFF = tuple(sum(WO_ROWS[:i]) for i in range(WOC + 1))
assert WO_OFF[-1] == HQ * DH


def _kernel(x_h, k_h, v_h, wq_h, wo_h, w1_h, b1_h, w2_h, b2_h, gw_h,
            o_ref,
            xb, b1b, b2b, gwb, wqb, wob, w1b, w2b, kb, vb,
            q_s, o_s, sem):
    def sem_of(stage):
        return sem.at[stage % NSEM]

    def kv_copies(u):
        h, b, slot = u // B, u % B, u % NSLOT
        s = sem_of(u + PRE)
        return (pltpu.make_async_copy(k_h.at[b, h], kb.at[slot], s),
                pltpu.make_async_copy(v_h.at[b, h], vb.at[slot], s))

    stage0 = [pltpu.make_async_copy(src, dst, sem_of(0)) for src, dst in
              ((wq_h, wqb), (x_h, xb), (b1_h, b1b), (b2_h, b2b), (gw_h, gwb))]
    stage1 = [pltpu.make_async_copy(src, dst, sem_of(1)) for src, dst in
              ((w1_h, w1b), (w2_h, w2b))]

    def wo_copy(c):
        rows = pl.ds(WO_OFF[c], WO_ROWS[c])
        return pltpu.make_async_copy(wo_h.at[rows], wob.at[rows], sem_of(PRE + NU + c))

    def start_stage(i):
        if i == 0:
            copies = stage0
        elif i == 1:
            copies = stage1
        elif i < PRE + NU:
            copies = kv_copies(i - PRE)
        elif i < PRE + NU + WOC:
            copies = (wo_copy(i - PRE - NU),)
        else:
            copies = ()
        for c in copies:
            c.start()

    for i in range(NSEM):
        start_stage(i)

    for c in stage0:
        c.wait()
    start_stage(0 + NSEM)

    x4 = xb[...].astype(jnp.float32)
    x16b = jnp.concatenate([x4] * REP, axis=0).astype(jnp.bfloat16)
    row = lax.broadcasted_iota(jnp.int32, (M, DH), 0)
    for h in range(HKV):
        qh = jnp.dot(x16b, wqb[:, h * REP * DH:(h + 1) * REP * DH],
                     preferred_element_type=jnp.float32)
        sel = qh[:, 0:DH]
        for r in range(1, REP):
            sel = jnp.where(row // B == r, qh[:, r * DH:(r + 1) * DH], sel)
        q_s[h] = sel.astype(jnp.bfloat16)

    gate_logit = jnp.sum(x4 * gwb[...].astype(jnp.float32).reshape(1, D),
                         axis=1, keepdims=True)
    g = jax.nn.sigmoid(gate_logit)

    for c in stage1:
        c.wait()
    start_stage(1 + NSEM)

    hid = jnp.dot(x16b, w1b[...], preferred_element_type=jnp.float32)
    hid = hid + b1b[...].astype(jnp.float32).reshape(1, F)
    hid = hid.astype(jnp.bfloat16).astype(jnp.float32)
    hid = jnp.maximum(hid, 0.0)
    hid = (hid * hid).astype(jnp.bfloat16)
    ffn = jnp.dot(hid, w2b[...], preferred_element_type=jnp.float32)[0:B]
    ffn = ffn + b2b[...].astype(jnp.float32).reshape(1, D)
    base = (1.0 - g) * ffn

    c_exp = (DH ** -0.5) * LOG2E

    def unit(u, carry):
        h, b, slot = u // B, u % B, u % NSLOT
        for c in kv_copies(u):
            c.wait()

        nxt = u + NSEM

        @pl.when(nxt < NU)
        def _():
            for c in kv_copies(nxt):
                c.start()

        for c in range(min(WOC, NSEM)):
            @pl.when(nxt - NU == c)
            def _():
                wo_copy(c).start()

        s = lax.dot_general(q_s[h], kb[slot], (((1,), (1,)), ((), ())),
                            preferred_element_type=jnp.float32)
        m = jnp.max(s, axis=1, keepdims=True)
        p = jnp.exp2((s - m) * c_exp)
        l = jnp.sum(p, axis=1, keepdims=True)
        o = jnp.dot(p.astype(jnp.bfloat16), vb[slot],
                    preferred_element_type=jnp.float32) / l

        @pl.when(b == 0)
        def _():
            o_s[h] = o

        @pl.when(b > 0)
        def _():
            o_s[h] = jnp.where(row % B == b, o, o_s[h])

        return carry

    lax.fori_loop(0, NU, unit, 0)

    pieces = []
    for h in range(HKV):
        oh = o_s[h]
        for r in range(REP):
            pieces.append(oh[r * B:(r + 1) * B, :])
    attn = jnp.concatenate(pieces, axis=1).astype(jnp.bfloat16)

    acc = None
    for c in range(WOC):
        lhs = attn[:, WO_OFF[c]:WO_OFF[c + 1]]
        wo_copy(c).wait()
        start_stage(PRE + NU + c + NSEM)
        part = jnp.dot(lhs, wob[WO_OFF[c]:WO_OFF[c + 1], :],
                       preferred_element_type=jnp.float32)
        acc = part if acc is None else acc + part

    o_ref[...] = (g * acc + base).astype(o_ref.dtype)


@jax.jit
def pallas_gated_mix__gqa_block_cached__dense_activation_squared_relu__decode_kernel(
    A_x: jax.Array,
    A_k_cache: jax.Array,
    A_v_cache: jax.Array,
    A_wq: jax.Array,
    A_wo: jax.Array,
    B_x: jax.Array,
    B_w1: jax.Array,
    B_b1: jax.Array,
    B_w2: jax.Array,
    B_b2: jax.Array,
    gate_w: jax.Array,
):
    del B_x
    bf16, f32 = jnp.bfloat16, jnp.float32
    out = pl.pallas_call(
        _kernel,
        out_shape=jax.ShapeDtypeStruct((B, D), bf16),
        in_specs=[pl.BlockSpec(memory_space=pl.ANY)] * 10,
        out_specs=pl.BlockSpec(memory_space=pltpu.VMEM),
        scratch_shapes=[
            pltpu.VMEM((B, D), bf16),
            pltpu.VMEM((F,), bf16),
            pltpu.VMEM((D,), bf16),
            pltpu.VMEM((D,), bf16),
            pltpu.VMEM((D, HQ * DH), bf16),
            pltpu.VMEM((HQ * DH, D), bf16),
            pltpu.VMEM((D, F), bf16),
            pltpu.VMEM((F, D), bf16),
            pltpu.VMEM((NSLOT, SK, DH), bf16),
            pltpu.VMEM((NSLOT, SK, DH), bf16),
            pltpu.VMEM((HKV, M, DH), bf16),
            pltpu.VMEM((HKV, M, DH), f32),
            pltpu.SemaphoreType.DMA((NSEM,)),
        ],
        compiler_params=pltpu.CompilerParams(vmem_limit_bytes=64 * 1024 * 1024),
    )(A_x.reshape(B, D), A_k_cache, A_v_cache, A_wq, A_wo, B_w1, B_b1, B_w2, B_b2, gate_w)
    return out.reshape(B, 1, D)
```

```python
import jax
import jax.numpy as jnp
from jax import lax
import jax.experimental.pallas as pl
import jax.experimental.pallas.tpu as pltpu

B, D, HQ, HKV, SK, DH, F = 4, 512, 32, 8, 4096, 128, 1792
REP = HQ // HKV
M = REP * B
LOG2E = 1.4426950408889634

NSEM = 3
NSLOT = NSEM + 1
NU = HKV * B
PRE = 2

WO_ROWS = (1664, 1024, 640, 384, 256, 128)
KV_PIECE, KV_SEGS = 160, 4
WQ_PIECE, WQ_SEGS = 2048, 6
W1_PIECE, W2_PIECE, W12_SEGS = 8, 40, 4
WO_PIECE, WO_SEGS = 40, 4

WOC = len(WO_ROWS)
WO_OFF = tuple(sum(WO_ROWS[:i]) for i in range(WOC + 1))
assert WO_OFF[-1] == HQ * DH


def _cut(lo, hi, step):
    return [(r, min(step, hi - r)) for r in range(lo, hi, step)]


def _interleave(streams, nseg):
    segs = []
    for st in streams:
        per = -(-len(st) // nseg)
        segs += [st[i * per:(i + 1) * per] for i in range(nseg)]
    order = [s[j] for j in range(max(len(s) for s in segs)) for s in segs if j < len(s)]
    assert sorted(order) == sorted(p for st in streams for p in st)
    return [(p, i % 2) for i, p in enumerate(order)]


KV_PLAN = _interleave([[(t,) + p for p in _cut(0, SK, KV_PIECE)] for t in (0, 1)], KV_SEGS)
WQ_PLAN = _interleave([[(r, c) for r in range(0, D, 8) for c in range(0, HQ * DH, WQ_PIECE)]], WQ_SEGS)
W12_PLAN = _interleave([[(0,) + p for p in _cut(0, D, W1_PIECE)],
                        [(1,) + p for p in _cut(0, F, W2_PIECE)]], W12_SEGS)
WO_PLAN = [_interleave([_cut(WO_OFF[c], WO_OFF[c + 1], WO_PIECE)], WO_SEGS) for c in range(WOC)]


def _kernel(x_h, k_h, v_h, wq_h, wo_h, w1_h, b1_h, w2_h, b2_h, gw_h,
            o_ref,
            xb, b1b, b2b, gwb, wqb, wob, w1b, w2b, kb, vb,
            q_s, o_s, sem):
    def sem_of(stage):
        return sem.at[stage % NSEM]

    def wait_all(region, s):
        pltpu.make_async_copy(region, region, s).wait()

    small = [pltpu.make_async_copy(src, dst, sem_of(0)) for src, dst in
             ((x_h, xb), (b1_h, b1b), (b2_h, b2b), (gw_h, gwb))]

    def wq_start():
        for c in small:
            c.start()
        for (r, c), prio in WQ_PLAN:
            idx = (pl.ds(r, 8), pl.ds(c, WQ_PIECE))
            pltpu.make_async_copy(wq_h.at[idx], wqb.at[idx], sem_of(0)).start(priority=prio)

    def wq_wait():
        for c in small:
            c.wait()
        wait_all(wqb, sem_of(0))

    def w12_start():
        for (t, r, n), prio in W12_PLAN:
            src, dst = ((w1_h, w1b), (w2_h, w2b))[t]
            pltpu.make_async_copy(src.at[pl.ds(r, n)], dst.at[pl.ds(r, n)],
                                  sem_of(1)).start(priority=prio)

    def w12_wait():
        wait_all(w1b, sem_of(1))
        wait_all(w2b, sem_of(1))

    def kv_start(u):
        h, b, slot = u // B, u % B, u % NSLOT
        for (t, r, n), prio in KV_PLAN:
            src, dst = ((k_h, kb), (v_h, vb))[t]
            pltpu.make_async_copy(src.at[b, h, pl.ds(r, n)], dst.at[slot, pl.ds(r, n)],
                                  sem_of(u + PRE)).start(priority=prio)

    def kv_wait(u):
        wait_all(kb.at[u % NSLOT], sem_of(u + PRE))
        wait_all(vb.at[u % NSLOT], sem_of(u + PRE))

    def wo_start(c):
        for (r, n), prio in WO_PLAN[c]:
            pltpu.make_async_copy(wo_h.at[pl.ds(r, n)], wob.at[pl.ds(r, n)],
                                  sem_of(PRE + NU + c)).start(priority=prio)

    def wo_wait(c):
        wait_all(wob.at[pl.ds(WO_OFF[c], WO_ROWS[c])], sem_of(PRE + NU + c))

    def start_stage(i):
        if i == 0:
            wq_start()
        elif i == 1:
            w12_start()
        elif i < PRE + NU:
            kv_start(i - PRE)
        elif i < PRE + NU + WOC:
            wo_start(i - PRE - NU)

    for i in range(NSEM):
        start_stage(i)

    wq_wait()
    start_stage(0 + NSEM)

    x4 = xb[...].astype(jnp.float32)
    x16b = jnp.concatenate([x4] * REP, axis=0).astype(jnp.bfloat16)
    row = lax.broadcasted_iota(jnp.int32, (M, DH), 0)
    for h in range(HKV):
        qh = jnp.dot(x16b, wqb[:, h * REP * DH:(h + 1) * REP * DH],
                     preferred_element_type=jnp.float32)
        sel = qh[:, 0:DH]
        for r in range(1, REP):
            sel = jnp.where(row // B == r, qh[:, r * DH:(r + 1) * DH], sel)
        q_s[h] = sel.astype(jnp.bfloat16)

    gate_logit = jnp.sum(x4 * gwb[...].astype(jnp.float32).reshape(1, D),
                         axis=1, keepdims=True)
    g = jax.nn.sigmoid(gate_logit)

    w12_wait()
    start_stage(1 + NSEM)

    hid = jnp.dot(x16b, w1b[...], preferred_element_type=jnp.float32)
    hid = hid + b1b[...].astype(jnp.float32).reshape(1, F)
    hid = hid.astype(jnp.bfloat16).astype(jnp.float32)
    hid = jnp.maximum(hid, 0.0)
    hid = (hid * hid).astype(jnp.bfloat16)
    ffn = jnp.dot(hid, w2b[...], preferred_element_type=jnp.float32)[0:B]
    ffn = ffn + b2b[...].astype(jnp.float32).reshape(1, D)
    base = (1.0 - g) * ffn

    c_exp = (DH ** -0.5) * LOG2E

    def unit(u, carry):
        h, b, slot = u // B, u % B, u % NSLOT
        kv_wait(u)

        nxt = u + NSEM

        @pl.when(nxt < NU)
        def _():
            kv_start(nxt)

        for c in range(min(WOC, NSEM)):
            @pl.when(nxt - NU == c)
            def _():
                wo_start(c)

        s = lax.dot_general(q_s[h], kb[slot], (((1,), (1,)), ((), ())),
                            preferred_element_type=jnp.float32)
        m = jnp.max(s, axis=1, keepdims=True)
        p = jnp.exp2((s - m) * c_exp)
        l = jnp.sum(p, axis=1, keepdims=True)
        o = jnp.dot(p.astype(jnp.bfloat16), vb[slot],
                    preferred_element_type=jnp.float32) / l

        @pl.when(b == 0)
        def _():
            o_s[h] = o

        @pl.when(b > 0)
        def _():
            o_s[h] = jnp.where(row % B == b, o, o_s[h])

        return carry

    lax.fori_loop(0, NU, unit, 0)

    pieces = []
    for h in range(HKV):
        oh = o_s[h]
        for r in range(REP):
            pieces.append(oh[r * B:(r + 1) * B, :])
    attn = jnp.concatenate(pieces, axis=1).astype(jnp.bfloat16)

    acc = None
    for c in range(WOC):
        lhs = attn[:, WO_OFF[c]:WO_OFF[c + 1]]
        wo_wait(c)
        start_stage(PRE + NU + c + NSEM)
        part = jnp.dot(lhs, wob[WO_OFF[c]:WO_OFF[c + 1], :],
                       preferred_element_type=jnp.float32)
        acc = part if acc is None else acc + part

    o_ref[...] = (g * acc + base).astype(o_ref.dtype)


@jax.jit
def pallas_gated_mix__gqa_block_cached__dense_activation_squared_relu__decode_kernel(
    A_x: jax.Array,
    A_k_cache: jax.Array,
    A_v_cache: jax.Array,
    A_wq: jax.Array,
    A_wo: jax.Array,
    B_x: jax.Array,
    B_w1: jax.Array,
    B_b1: jax.Array,
    B_w2: jax.Array,
    B_b2: jax.Array,
    gate_w: jax.Array,
):
    del B_x
    bf16, f32 = jnp.bfloat16, jnp.float32
    out = pl.pallas_call(
        _kernel,
        out_shape=jax.ShapeDtypeStruct((B, D), bf16),
        in_specs=[pl.BlockSpec(memory_space=pl.ANY)] * 10,
        out_specs=pl.BlockSpec(memory_space=pltpu.VMEM),
        scratch_shapes=[
            pltpu.VMEM((B, D), bf16),
            pltpu.VMEM((F,), bf16),
            pltpu.VMEM((D,), bf16),
            pltpu.VMEM((D,), bf16),
            pltpu.VMEM((D, HQ * DH), bf16),
            pltpu.VMEM((HQ * DH, D), bf16),
            pltpu.VMEM((D, F), bf16),
            pltpu.VMEM((F, D), bf16),
            pltpu.VMEM((NSLOT, SK, DH), bf16),
            pltpu.VMEM((NSLOT, SK, DH), bf16),
            pltpu.VMEM((HKV, M, DH), bf16),
            pltpu.VMEM((HKV, M, DH), f32),
            pltpu.SemaphoreType.DMA((NSEM,)),
        ],
        compiler_params=pltpu.CompilerParams(vmem_limit_bytes=64 * 1024 * 1024),
    )(A_x.reshape(B, D), A_k_cache, A_v_cache, A_wq, A_wo, B_w1, B_b1, B_w2, B_b2, gate_w)
    return out.reshape(B, 1, D)
```

```python
import jax
import jax.numpy as jnp
from jax import lax
import jax.experimental.pallas as pl
import jax.experimental.pallas.tpu as pltpu

B, D, HQ, HKV, SK, DH, F = 4, 512, 32, 8, 4096, 128, 1792
REP = HQ // HKV
M = REP * B
LOG2E = 1.4426950408889634

NSEM = 3
NSLOT = NSEM + 1
UPS = 2
NST = HKV * B // UPS
PRE = 2

WO_ROWS = (1536, 1024, 768, 384, 256, 128)
KV_PIECE = 128
KV_SPLIT = 2176
WQ_PIECE, WQ_SEGS = 1024, 8
W1_PIECE, W2_PIECE, W12_SEGS = 8, 32, 4
WO_PIECE, WO_SEGS = 32, 4

WOC = len(WO_ROWS)
WO_OFF = tuple(sum(WO_ROWS[:i]) for i in range(WOC + 1))
assert WO_OFF[-1] == HQ * DH


def _cut(lo, hi, step):
    return [(r, min(step, hi - r)) for r in range(lo, hi, step)]


def _split(pieces, nseg):
    per = -(-len(pieces) // nseg)
    return [pieces[i * per:(i + 1) * per] for i in range(nseg)]


def _interleave(segs):
    order = [s[j] for j in range(max(len(s) for s in segs)) for s in segs if j < len(s)]
    assert len(order) == sum(len(s) for s in segs)
    return [(p, i % 2) for i, p in enumerate(order)]


KV_PLAN = _interleave([[(g, t) + p for p in _cut(lo, hi, KV_PIECE)]
                       for lo, hi in ((0, KV_SPLIT), (KV_SPLIT, SK))
                       for g in range(UPS) for t in (0, 1)])
WQ_PLAN = _interleave(_split([(r, c) for r in range(0, D, 8)
                              for c in range(0, HQ * DH, WQ_PIECE)], WQ_SEGS))
W12_PLAN = _interleave(_split([(0,) + p for p in _cut(0, D, W1_PIECE)], W12_SEGS)
                       + _split([(1,) + p for p in _cut(0, F, W2_PIECE)], W12_SEGS))
WO_PLAN = [_interleave(_split(_cut(WO_OFF[c], WO_OFF[c + 1], WO_PIECE), WO_SEGS))
           for c in range(WOC)]
assert (HQ * DH) % WQ_PIECE == 0


def _kernel(x_h, k_h, v_h, wq_h, wo_h, w1_h, b1_h, w2_h, b2_h, gw_h,
            o_ref,
            xb, b1b, b2b, gwb, wqb, wob, w1b, w2b, kb, vb,
            q_s, o_s, sem):
    def sem_of(stage):
        return sem.at[stage % NSEM]

    def wait_all(region, s):
        pltpu.make_async_copy(region, region, s).wait()

    small = [pltpu.make_async_copy(src, dst, sem_of(0)) for src, dst in
             ((x_h, xb), (b1_h, b1b), (b2_h, b2b), (gw_h, gwb))]

    def wq_start():
        for c in small:
            c.start()
        for (r, c), prio in WQ_PLAN:
            idx = (pl.ds(r, 8), pl.ds(c, WQ_PIECE))
            pltpu.make_async_copy(wq_h.at[idx], wqb.at[idx], sem_of(0)).start(priority=prio)

    def wq_wait():
        for c in small:
            c.wait()
        wait_all(wqb, sem_of(0))

    def w12_start():
        for (t, r, n), prio in W12_PLAN:
            src, dst = ((w1_h, w1b), (w2_h, w2b))[t]
            pltpu.make_async_copy(src.at[pl.ds(r, n)], dst.at[pl.ds(r, n)],
                                  sem_of(1)).start(priority=prio)

    def w12_wait():
        wait_all(w1b, sem_of(1))
        wait_all(w2b, sem_of(1))

    def kv_start(st):
        for (g, t, r, n), prio in KV_PLAN:
            u = st * UPS + g
            src, dst = ((k_h, kb), (v_h, vb))[t]
            pltpu.make_async_copy(src.at[u % B, u // B, pl.ds(r, n)],
                                  dst.at[st % NSLOT, g, pl.ds(r, n)],
                                  sem_of(PRE + st)).start(priority=prio)

    def kv_wait(st):
        wait_all(kb.at[st % NSLOT], sem_of(PRE + st))
        wait_all(vb.at[st % NSLOT], sem_of(PRE + st))

    def wo_start(c):
        for (r, n), prio in WO_PLAN[c]:
            pltpu.make_async_copy(wo_h.at[pl.ds(r, n)], wob.at[pl.ds(r, n)],
                                  sem_of(PRE + NST + c)).start(priority=prio)

    def wo_wait(c):
        wait_all(wob.at[pl.ds(WO_OFF[c], WO_ROWS[c])], sem_of(PRE + NST + c))

    def start_stage(i):
        if i == 0:
            wq_start()
        elif i == 1:
            w12_start()
        elif i < PRE + NST:
            kv_start(i - PRE)
        elif i < PRE + NST + WOC:
            wo_start(i - PRE - NST)

    for i in range(NSEM):
        start_stage(i)

    wq_wait()
    start_stage(0 + NSEM)

    x4 = xb[...].astype(jnp.float32)
    x16b = jnp.concatenate([x4] * REP, axis=0).astype(jnp.bfloat16)
    row = lax.broadcasted_iota(jnp.int32, (M, DH), 0)
    for h in range(HKV):
        qh = jnp.dot(x16b, wqb[:, h * REP * DH:(h + 1) * REP * DH],
                     preferred_element_type=jnp.float32)
        sel = qh[:, 0:DH]
        for r in range(1, REP):
            sel = jnp.where(row // B == r, qh[:, r * DH:(r + 1) * DH], sel)
        q_s[h] = sel.astype(jnp.bfloat16)

    gate_logit = jnp.sum(x4 * gwb[...].astype(jnp.float32).reshape(1, D),
                         axis=1, keepdims=True)
    gate = jax.nn.sigmoid(gate_logit)

    w12_wait()
    start_stage(1 + NSEM)

    hid = jnp.dot(x16b, w1b[...], preferred_element_type=jnp.float32)
    hid = hid + b1b[...].astype(jnp.float32).reshape(1, F)
    hid = hid.astype(jnp.bfloat16).astype(jnp.float32)
    hid = jnp.maximum(hid, 0.0)
    hid = (hid * hid).astype(jnp.bfloat16)
    ffn = jnp.dot(hid, w2b[...], preferred_element_type=jnp.float32)[0:B]
    ffn = ffn + b2b[...].astype(jnp.float32).reshape(1, D)
    base = (1.0 - gate) * ffn

    c_exp = (DH ** -0.5) * LOG2E

    def attention_stage(st, carry):
        kv_wait(st)

        nxt = st + NSEM

        @pl.when(nxt < NST)
        def _():
            kv_start(nxt)

        for c in range(min(WOC, NSEM)):
            @pl.when(nxt - NST == c)
            def _():
                wo_start(c)

        for g in range(UPS):
            u = st * UPS + g
            h, b = u // B, u % B
            s = lax.dot_general(q_s[h], kb[st % NSLOT, g], (((1,), (1,)), ((), ())),
                                preferred_element_type=jnp.float32)
            m = jnp.max(s, axis=1, keepdims=True)
            p = jnp.exp2((s - m) * c_exp)
            l = jnp.sum(p, axis=1, keepdims=True)
            o = jnp.dot(p.astype(jnp.bfloat16), vb[st % NSLOT, g],
                        preferred_element_type=jnp.float32) / l

            @pl.when(b == 0)
            def _():
                o_s[h] = o

            @pl.when(b > 0)
            def _():
                o_s[h] = jnp.where(row % B == b, o, o_s[h])

        return carry

    lax.fori_loop(0, NST, attention_stage, 0)

    pieces = []
    for h in range(HKV):
        oh = o_s[h]
        for r in range(REP):
            pieces.append(oh[r * B:(r + 1) * B, :])
    attn = jnp.concatenate(pieces, axis=1).astype(jnp.bfloat16)

    acc = None
    for c in range(WOC):
        lhs = attn[:, WO_OFF[c]:WO_OFF[c + 1]]
        wo_wait(c)
        start_stage(PRE + NST + c + NSEM)
        part = jnp.dot(lhs, wob[WO_OFF[c]:WO_OFF[c + 1], :],
                       preferred_element_type=jnp.float32)
        acc = part if acc is None else acc + part

    o_ref[...] = (gate * acc + base).astype(o_ref.dtype)


@jax.jit
def pallas_gated_mix__gqa_block_cached__dense_activation_squared_relu__decode_kernel(
    A_x: jax.Array,
    A_k_cache: jax.Array,
    A_v_cache: jax.Array,
    A_wq: jax.Array,
    A_wo: jax.Array,
    B_x: jax.Array,
    B_w1: jax.Array,
    B_b1: jax.Array,
    B_w2: jax.Array,
    B_b2: jax.Array,
    gate_w: jax.Array,
):
    del B_x
    bf16, f32 = jnp.bfloat16, jnp.float32
    out = pl.pallas_call(
        _kernel,
        out_shape=jax.ShapeDtypeStruct((B, D), bf16),
        in_specs=[pl.BlockSpec(memory_space=pl.ANY)] * 10,
        out_specs=pl.BlockSpec(memory_space=pltpu.VMEM),
        scratch_shapes=[
            pltpu.VMEM((B, D), bf16),
            pltpu.VMEM((F,), bf16),
            pltpu.VMEM((D,), bf16),
            pltpu.VMEM((D,), bf16),
            pltpu.VMEM((D, HQ * DH), bf16),
            pltpu.VMEM((HQ * DH, D), bf16),
            pltpu.VMEM((D, F), bf16),
            pltpu.VMEM((F, D), bf16),
            pltpu.VMEM((NSLOT, UPS, SK, DH), bf16),
            pltpu.VMEM((NSLOT, UPS, SK, DH), bf16),
            pltpu.VMEM((HKV, M, DH), bf16),
            pltpu.VMEM((HKV, M, DH), f32),
            pltpu.SemaphoreType.DMA((NSEM,)),
        ],
        compiler_params=pltpu.CompilerParams(vmem_limit_bytes=64 * 1024 * 1024),
    )(A_x.reshape(B, D), A_k_cache, A_v_cache, A_wq, A_wo, B_w1, B_b1, B_w2, B_b2, gate_w)
    return out.reshape(B, 1, D)
```
